```python
import os as _os
_os.environ.setdefault("JAX_PLATFORMS", "cpu")
import jax
import jax.numpy as jnp

def _softmax(x, axis=-1):
    return jax.nn.softmax(x, axis=axis)
def _gelu(x):
    return jax.nn.gelu(x, approximate=True)
def _silu(x):
    return jax.nn.silu(x)
def _sigmoid(x):
    return jax.nn.sigmoid(x)
def _layernorm(x, axis=-1, eps=1e-5):
    m = jnp.mean(x, axis=axis, keepdims=True)
    v = jnp.var(x, axis=axis, keepdims=True)
    return (x - m) / jnp.sqrt(v + eps)
def _scatter_add(tgt, idx, src, axis=0):
    return tgt.at[idx].add(src)
def _segment_sum(src, seg, n):
    return jax.ops.segment_sum(src, seg, n)
class _Rng:
    def __init__(self, key):
        self._k = key
    def _next(self):
        self._k, sub = jax.random.split(self._k)
        return sub
    def normal(self, shape):
        return jax.random.normal(self._next(), shape, dtype=jnp.bfloat16)
    def randint(self, lo, hi, shape):
        return jax.random.randint(self._next(), shape, lo, hi, dtype=jnp.int32)
    def uniform(self, shape, lo=0.0, hi=1.0):
        return jax.random.uniform(self._next(), shape, jnp.bfloat16, lo, hi)
    def permutation(self, n):
        return jax.random.permutation(self._next(), n)


kernel_name = 'recurrent_scan__grouped_kv_mqa__mixer_s_mlp__prompt'

def setup_inputs():
    _rng = _Rng(jax.random.key(int.from_bytes(__import__("os").urandom(4), "little")))
    _w = (lambda a: (lambda t: t.astype(jnp.bfloat16) if jnp.issubdtype(t.dtype, jnp.floating) else t)(jnp.asarray(a)))
    def _A_setup():
        B, S, D, H = 1, 2048, 512, 32
        Dh = D // H
        return {
            "x": _w((lambda *s: _rng.normal(s) * 0.05)(B, S, D)),
            "wq": _w((lambda *s: _rng.normal(s) * 0.05)(D, H * Dh)),
            "wk": _w((lambda *s: _rng.normal(s) * 0.05)(D, Dh)),
            "wv": _w((lambda *s: _rng.normal(s) * 0.05)(D, Dh)),
            "wo": _w((lambda *s: _rng.normal(s) * 0.05)(H * Dh, D)),
        }
    _A_in = _A_setup()

    def _B_setup():
        B, S, D, F = 1, 2048, 512, 1792
        return {
            "x":  _w((lambda *s: _rng.normal(s) * 0.05)(B, S, D)),
            "w1": _w((lambda *s: _rng.normal(s) * 0.8)(D, D) * (D ** -0.5)),
            "w2": _w((lambda *s: _rng.normal(s) * 0.8)(D, D) * (D ** -0.5)),
            "w3": _w((lambda *s: _rng.normal(s) * 0.8)(D, F) * (D ** -0.5)),
            "w4": _w((lambda *s: _rng.normal(s) * 0.8)(F, D) * (F ** -0.5)),
        }
    _B_in = _B_setup()

    return {
        "A_x": _A_in["x"],
        "A_wq": _A_in["wq"],
        "A_wk": _A_in["wk"],
        "A_wv": _A_in["wv"],
        "A_wo": _A_in["wo"],
        "B_x": _B_in["x"],
        "B_w1": _B_in["w1"],
        "B_w2": _B_in["w2"],
        "B_w3": _B_in["w3"],
        "B_w4": _B_in["w4"],
    }

def reference(A_x, A_wq, A_wk, A_wv, A_wo, B_x, B_w1, B_w2, B_w3, B_w4):
    def _A_ref(x, wq, wk, wv, wo):
        B, S, D = x.shape
        H = 32
        Dh = D // H
        q = (lambda x, *d: x.transpose(*d))((x @ wq).reshape(B, S, H, Dh), 0, 2, 1, 3)
        k = x @ wk
        v = x @ wv
        scores = jnp.einsum("bhqd,bkd->bhqk", q, k) * (Dh ** -0.5)
        p = _softmax(scores, axis=-1)
        o = jnp.einsum("bhqk,bkd->bhqd", p, v)
        return (lambda x, *d: x.transpose(*d))(o, 0, 2, 1, 3).reshape(B, S, H * Dh) @ wo

    def _B_ref(x, w1, w2, w3, w4):
        B, S, D = x.shape
        h = _gelu(_layernorm(x, axis=-1) @ w1)
        c = D // 4
        g0 = jnp.pad(h[:, :, 0*c:1*c], ((0, 0), (1, 0), (0, 0)))[:, :S, :]
        g1 = jnp.pad(h[:, :, 1*c:2*c], ((0, 0), (0, 1), (0, 0)))[:, 1:, :]
        g2 = jnp.pad(h[:, :, 2*c:3*c], ((0, 0), (2, 0), (0, 0)))[:, :S, :]
        g3 = jnp.pad(h[:, :, 3*c:   ], ((0, 0), (0, 2), (0, 0)))[:, 2:, :]
        hs = jnp.concatenate([g0, g1, g2, g3], axis=-1) @ w2
        x1 = x + hs
        h2 = _gelu(_layernorm(x1, axis=-1) @ w3) @ w4
        return x1 + h2

    x = A_x
    xn = _layernorm(x, axis=-1)
    s = _A_ref(xn, A_wq, A_wk, A_wv, A_wo)
    g = _silu(_B_ref(xn, B_w1, B_w2, B_w3, B_w4))
    return x + s * g
```

```python
import functools

import numpy as np
import jax
import jax.numpy as jnp
import jax.experimental.pallas as pl
import jax.experimental.pallas.tpu as pltpu

S, D, H, DH, F = 2048, 512, 32, 16, 1792
RB = 512
NB = S // RB
CK = 128
PAD = 8
EPS = 1e-5
QSCALE = float(DH ** -0.5 * np.log2(np.e))
f32, bf16 = jnp.float32, jnp.bfloat16

_NT = (((1,), (1,)), ((), ()))
_TN = (((0,), (0,)), ((), ()))


def _ln(x):
    m = jnp.mean(x, axis=-1, keepdims=True)
    d = x - m
    v = jnp.mean(d * d, axis=-1, keepdims=True)
    return d * jax.lax.rsqrt(v + EPS)


def _gelu(x):
    c0 = float(np.sqrt(2.0 / np.pi))
    c1 = c0 * 0.044715
    hx = 0.5 * x
    return hx + hx * jnp.tanh(x * (c0 + c1 * (x * x)))


def _dot(a, b):
    return jnp.dot(a, b, preferred_element_type=f32)


def _kernel(x_h, wq_h, wkt_h, wvt_h, wo_h, w1_h, w2_h, w3_h, w4_h, out_h,
            x_v, wq_v, wkt_v, wvt_v, wo_v, w1_v, w2_v, w3_v, w4_v, out_v,
            wqt_s, xn_s, h_s, k_s, vt_s, qt_s, ot_s, sbuf, xsem, wsem, osem):
    def x_copy(b):
        r = pl.ds(b * RB, RB)
        return pltpu.make_async_copy(x_h.at[r], x_v.at[r], xsem.at[b])

    w_pairs = [(wq_h, wq_v), (wkt_h, wkt_v), (wvt_h, wvt_v), (w1_h, w1_v),
               (wo_h, wo_v), (w2_h, w2_v), (w3_h, w3_v), (w4_h, w4_v)]
    w_copies = [pltpu.make_async_copy(s, d, wsem.at[i]) for i, (s, d) in enumerate(w_pairs)]

    x_copy(0).start()
    for c in w_copies[:4]:
        c.start()
    for b in range(1, NB):
        x_copy(b).start()
    for c in w_copies[4:]:
        c.start()

    h_s[0:PAD, :] = jnp.zeros((PAD, D), f32)
    h_s[PAD + S:PAD + S + PAD, :] = jnp.zeros((PAD, D), f32)

    for c in w_copies[:4]:
        c.wait()
    wqt_s[...] = (wq_v[...].astype(f32).T).astype(bf16)

    def proj(b, _):
        x_copy(b).wait()
        r0 = pl.multiple_of(b * RB, RB)
        rows = pl.ds(r0, RB)
        xn = _ln(x_v[rows, :].astype(f32))
        xn_s[rows, :] = xn
        xb = xn.astype(bf16)
        qt = jax.lax.dot_general(wqt_s[...], xb, _NT, preferred_element_type=f32)
        qt_s[b] = (qt * QSCALE).astype(bf16)
        vt_s[b] = jax.lax.dot_general(wvt_v[...], xb, _NT, preferred_element_type=f32).astype(bf16)
        k_s[rows, :] = jax.lax.dot_general(xb, wkt_v[...], _NT, preferred_element_type=f32).astype(bf16)
        h_s[pl.ds(pl.multiple_of(r0 + PAD, PAD), RB), :] = _gelu(_dot(_ln(xn).astype(bf16), w1_v[...]))
        return 0

    jax.lax.fori_loop(0, NB, proj, 0)

    NC = S // CK
    NT = NB * H

    def qk(t, slot, c, m):
        qt = qt_s[t // H, pl.ds(pl.multiple_of((t % H) * DH, DH), DH), :]
        s = _dot(k_s[c * CK:(c + 1) * CK, :], qt)
        sbuf[slot, c * CK:(c + 1) * CK, :] = s
        mm = jnp.max(s.reshape(CK // 8, 8, RB), axis=0)
        return mm if m is None else jnp.maximum(m, mm)

    def pv(slot, c, mb, l, acc):
        p = jnp.exp2(sbuf[slot, c * CK:(c + 1) * CK, :] - mb)
        ls = jnp.sum(p.reshape(CK // 8, 8, RB), axis=0)
        o = (c * CK) % RB
        a = _dot(vt_s[(c * CK) // RB, :, o:o + CK], p.astype(bf16))
        return (ls if l is None else l + ls), (a if acc is None else acc + a)

    m0 = None
    for c in range(NC):
        m0 = qk(0, 0, c, m0)

    def step(t, slot, m):
        mb = jnp.max(m, axis=0, keepdims=True)
        mn = l = acc = None
        tn = jnp.minimum(t + 1, NT - 1)
        for c in range(NC):
            mn = qk(tn, 1 - slot, c, mn)
            l, acc = pv(slot, c, mb, l, acc)
        lt = jnp.sum(l, axis=0, keepdims=True)
        ot_s[t // H, pl.ds(pl.multiple_of((t % H) * DH, DH), DH), :] = (acc * (1.0 / lt)).astype(bf16)
        return mn

    def attn(i, m):
        m = step(2 * i, 0, m)
        return step(2 * i + 1, 1, m)

    jax.lax.fori_loop(0, NT // 2, attn, m0)

    for c in w_copies[4:]:
        c.wait()

    def o_copy(b):
        r = pl.ds(b * RB, RB)
        return pltpu.make_async_copy(out_v.at[r], out_h.at[r], osem.at[b])

    def tail(b, _):
        r0 = pl.multiple_of(b * RB, RB)
        rows = pl.ds(r0, RB)
        g = D // 4
        parts = []
        for j, sh in enumerate((1, -1, 2, -2)):
            win = h_s[pl.ds(r0, RB + 2 * PAD), j * g:(j + 1) * g]
            parts.append(win[PAD - sh:PAD - sh + RB, :].astype(bf16))
        x1 = xn_s[rows, :] + _dot(jnp.concatenate(parts, axis=-1), w2_v[...])
        u = _gelu(_dot(_ln(x1).astype(bf16), w3_v[...])).astype(bf16)
        y = x1 + _dot(u, w4_v[...])
        gate = y * jax.nn.sigmoid(y)
        s = jax.lax.dot_general(ot_s[b], wo_v[...], _TN, preferred_element_type=f32)
        out_v[rows, :] = (x_v[rows, :].astype(f32) + s * gate).astype(bf16)
        o_copy(b).start()
        return 0

    jax.lax.fori_loop(0, NB, tail, 0)
    for b in range(NB):
        o_copy(b).wait()


@jax.jit
def pallas_recurrent_scan__grouped_kv_mqa__mixer_s_mlp__prompt_kernel(
    A_x: jax.Array,
    A_wq: jax.Array,
    A_wk: jax.Array,
    A_wv: jax.Array,
    A_wo: jax.Array,
    B_x: jax.Array,
    B_w1: jax.Array,
    B_w2: jax.Array,
    B_w3: jax.Array,
    B_w4: jax.Array,
):
    del B_x
    vm = pltpu.VMEM
    out = pl.pallas_call(
        _kernel,
        out_shape=jax.ShapeDtypeStruct((S, D), bf16),
        in_specs=[pl.BlockSpec(memory_space=pl.ANY)] * 9,
        out_specs=pl.BlockSpec(memory_space=pl.ANY),
        scratch_shapes=[
            vm((S, D), bf16), vm((D, D), bf16), vm((DH, D), bf16), vm((DH, D), bf16),
            vm((D, D), bf16), vm((D, D), bf16), vm((D, D), bf16), vm((D, F), bf16),
            vm((F, D), bf16), vm((S, D), bf16),
            vm((D, D), bf16),
            vm((S, D), f32),
            vm((S + 2 * PAD, D), f32),
            vm((S, DH), bf16),
            vm((NB, DH, RB), bf16),
            vm((NB, D, RB), bf16),
            vm((NB, D, RB), bf16),
            vm((2, S, RB), f32),
            pltpu.SemaphoreType.DMA((NB,)),
            pltpu.SemaphoreType.DMA((8,)),
            pltpu.SemaphoreType.DMA((NB,)),
        ],
        compiler_params=pltpu.CompilerParams(vmem_limit_bytes=100 * 1024 * 1024),
    )(A_x.reshape(S, D), A_wq, A_wk.T, A_wv.T, A_wo, B_w1, B_w2, B_w3, B_w4)
    return out.reshape(A_x.shape)
```

```python
import numpy as np
import jax
import jax.numpy as jnp
import jax.experimental.pallas as pl
import jax.experimental.pallas.tpu as pltpu

S, D, H, DH, F = 2048, 512, 32, 16, 1792
RB = 512
NB = S // RB
NT = NB * H
NL = RB // 128
CK = 128
NC = S // CK
PAD = 8
EPS = 1e-5
QSCALE = float(DH ** -0.5 * np.log2(np.e))

NV = 16
VCH = list(range(NC))
NG = len(VCH) * NV // 8
SCHED = [[g for g in range(NG) if g * NC // NG == c] for c in range(NC)]
UNROLL = 4
LAG = 2
PD = 3
HEADROOM = 64.0
FMAX = float(np.finfo(np.float32).max)

f32, bf16, u32 = jnp.float32, jnp.bfloat16, jnp.uint32
_NT_DIMS = (((1,), (1,)), ((), ()))
_TN_DIMS = (((0,), (0,)), ((), ()))


def _ln(x):
    m = jnp.mean(x, axis=-1, keepdims=True)
    d = x - m
    v = jnp.mean(d * d, axis=-1, keepdims=True)
    return d * jax.lax.rsqrt(v + EPS)


def _gelu(x):
    c0 = float(np.sqrt(2.0 / np.pi))
    c1 = c0 * 0.044715
    hx = 0.5 * x
    return hx + hx * jnp.tanh(x * (c0 + c1 * (x * x)))


def _dot(a, b):
    return jnp.dot(a, b, preferred_element_type=f32)


def _kernel(x_h, wq_h, wkt_h, wvt_h, wo_h, w1_h, w2_h, w3_h, w4_h, out_h,
            x_v, wq_v, wkt_v, wvt_v, wo_v, w1_v, w2_v, w3_v, w4_v, out_v,
            wt_s, xn_s, h_s, k_s, vt_s, qt_s, ot_s, qb_s, kb_s, p_s, sc_s,
            xsem, wsem, osem):
    def x_copy(b):
        r = pl.ds(b * RB, RB)
        return pltpu.make_async_copy(x_h.at[r], x_v.at[r], xsem.at[b])

    def o_copy(b):
        r = pl.ds(b * RB, RB)
        return pltpu.make_async_copy(out_v.at[r], out_h.at[r], osem.at[b])

    w_pairs = [(wq_h, wq_v), (wkt_h, wkt_v), (wvt_h, wvt_v), (w1_h, w1_v),
               (wo_h, wo_v), (w2_h, w2_v), (w3_h, w3_v), (w4_h, w4_v)]
    w_copies = [pltpu.make_async_copy(s, d, wsem.at[i]) for i, (s, d) in enumerate(w_pairs)]
    qkv_copies, w1_copy, late_copies = w_copies[:3], w_copies[3], w_copies[4:]

    x_copy(0).start()
    for cp in qkv_copies:
        cp.start()

    h_s[0:PAD, :] = jnp.zeros((PAD, D), f32)
    h_s[PAD + S:PAD + S + PAD, :] = jnp.zeros((PAD, D), f32)
    p_s[...] = jnp.zeros(p_s.shape, u32)

    def norm(b):
        x_copy(b).wait()
        if b == 0:
            x_copy(1).start()
            w1_copy.start()
        xn_s[b * RB:(b + 1) * RB, :] = _ln(x_v[b * RB:(b + 1) * RB, :].astype(f32))

    norm(0)
    for cp in qkv_copies:
        cp.wait()
    for b in range(2, NB):
        x_copy(b).start()
    for cp in late_copies:
        cp.start()
    wt_s[0:D] = (wq_v[...].astype(f32).T).astype(bf16)
    wt_s[D:D + DH] = wkt_v[...]
    wt_s[D + DH:] = wvt_v[...]

    ksq = None
    for b in range(NB):
        if b >= 1 and b + 1 < NB:
            norm(b + 1)
        xn = xn_s[b * RB:(b + 1) * RB, :]
        qkv = jax.lax.dot_general(wt_s[...], xn.astype(bf16), _NT_DIMS, preferred_element_type=f32)
        qt_s[b] = (qkv[0:D] * QSCALE).astype(bf16)
        vt_s[b] = pltpu.bitcast(qkv[D + DH:].astype(bf16), u32)
        kt = qkv[D:D + DH]
        n2 = jnp.sum(kt * kt, axis=0, keepdims=True)
        ksq = n2 if ksq is None else jnp.maximum(ksq, n2)
        ke = jnp.concatenate([kt, jnp.ones((1, RB), f32), jnp.zeros((127 - DH, RB), f32)], axis=0).T
        k_s[b * RB // 2:(b + 1) * RB // 2, :] = pltpu.bitcast(ke.astype(bf16), u32)
        if b == 0:
            norm(1)
            w1_copy.wait()
        h_s[PAD + b * RB:PAD + (b + 1) * RB, :] = _gelu(_dot(_ln(xn).astype(bf16), w1_v[...]))
    kmax = jnp.sqrt(jnp.max(ksq, axis=1, keepdims=True))

    def k_rows(r0, n, w):
        return pltpu.bitcast(k_s[r0 // 2:(r0 + n) // 2, :], bf16)[:, 0:w]

    for vi, c in enumerate(VCH):
        kf = k_rows((c + 1) * CK - NV, NV, DH).astype(f32)
        for d in range(DH):
            kb_s[d, vi * NV:(vi + 1) * NV, :] = jnp.broadcast_to(kf[:, d:d + 1], (NV, 128))

    def head_rows(t):
        return pl.ds(pl.multiple_of((t % H) * DH, DH), DH)

    def q_tile(t):
        return qt_s[t // H, head_rows(t), :]

    def vt_chunk(c):
        o = (c * CK) % RB
        return pltpu.bitcast(vt_s[(c * CK) // RB, :, o:o + CK], bf16)

    def finish(t, lt, acc):
        ot_s[t // H, head_rows(t), :] = (acc * (1.0 / lt)).astype(bf16)

    def neg_shift(t):
        qf = q_tile(t).astype(f32)
        return HEADROOM - jnp.sqrt(jnp.sum(qf * qf, axis=0, keepdims=True)) * kmax

    def check(ok, lt, acc):
        ok = jnp.where(jnp.abs(acc[0:8]) + jnp.abs(acc[8:16]) <= FMAX, ok, 0.0)
        return jnp.where((lt >= float(S)) & (lt <= FMAX), ok, 0.0)

    def fast(it, carry):
        lt, acc, ok, nxt = carry
        on = jnp.full((8, 128), it, jnp.int32) >= 0
        pend = [(NC - LAG + e, pltpu.bitcast(p_s[e], bf16)) for e in range(LAG)]
        for u in range(UNROLL):
            t = UNROLL * it + u
            qt = q_tile(t)
            qf = qt.astype(f32)
            sh = jnp.broadcast_to(nxt.astype(bf16), (DH, RB))
            nxt = neg_shift(jnp.minimum(t + 1, NT - 1))
            qe = jnp.concatenate([qt, sh], axis=0)
            shf = sh[0:8].astype(f32)
            for d in range(DH):
                qb_s[u % 2, d] = jnp.broadcast_to(qf[d:d + 1, :], (8, RB))
            l = None
            pvpu = {}
            for c in range(NC):
                nm = CK - NV if c in VCH else CK
                ng = nm // 16
                kl = jnp.concatenate(
                    [k_rows(c * CK + 16 * g, 16, 2 * DH) for g in reversed(range(ng))], axis=0)
                s = _dot(kl, qe)
                ps = []
                for j in range(nm // 8):
                    p = jnp.exp2(s[j * 8:(j + 1) * 8])
                    l = p if l is None else l + p
                    ps.append(p)
                if SCHED[c]:
                    parts = [[shf[:, n * 128:(n + 1) * 128] for n in range(NL)] for _ in SCHED[c]]
                    for d in range(DH):
                        qb = qb_s[u % 2, d]
                        j = d * (nm // 8) // DH
                        for a, g in enumerate(SCHED[c]):
                            kb = kb_s[d, g * 8:(g + 1) * 8, :]
                            if (d + a) % PD == 0:
                                kb = jnp.where(on, kb, s[j * 8:j * 8 + 8, 0:128])
                            for n in range(NL):
                                parts[a][n] = parts[a][n] + kb * qb[:, n * 128:(n + 1) * 128]
                    for a, g in enumerate(SCHED[c]):
                        pvpu[g] = jnp.exp2(jnp.concatenate(parts[a], axis=1))
                        l = l + pvpu[g]
                rows = []
                for g in reversed(range(ng)):
                    rows += ps[2 * g:2 * g + 2]
                if c in VCH:
                    g0 = VCH.index(c) * NV // 8
                    rows += [pvpu[g0 + i] for i in range(NV // 8)]
                pend.append((c, jnp.concatenate(rows, axis=0).astype(bf16)))
                cc, pb = pend.pop(0)
                a = _dot(vt_chunk(cc), pb)
                acc = a if cc == 0 else acc + a
                if cc == NC - 1:
                    finish(jnp.maximum(t - 1, 0), lt, acc)
                    ok = check(ok, lt, acc)
            lt = jnp.sum(l, axis=0, keepdims=True)
        for e, (_, pb) in enumerate(pend):
            p_s[e] = pltpu.bitcast(pb, u32)
        return lt, acc, ok, nxt

    lt, acc, ok, _ = jax.lax.fori_loop(
        0, NT // UNROLL, fast,
        (jnp.full((1, RB), float(S), f32), jnp.zeros((DH, RB), f32), jnp.ones((8, RB), f32),
         neg_shift(0)))
    for e in range(LAG):
        acc = acc + _dot(vt_chunk(NC - LAG + e), pltpu.bitcast(p_s[e], bf16))
    finish(NT - 1, lt, acc)
    ok = check(ok, lt, acc)

    @pl.when(jnp.min(ok) < 0.5)
    def _true_max_attention():
        def tile(t, _):
            qt = q_tile(t)

            def scores(b, m):
                kk = pltpu.bitcast(k_s[pl.ds(pl.multiple_of(b * (RB // 2), RB // 2), RB // 2), :], bf16)
                s = _dot(kk[:, 0:DH], qt)
                sc_s[b] = s
                return jnp.maximum(m, jnp.max(s, axis=0, keepdims=True))

            m = jax.lax.fori_loop(0, NB, scores, jnp.full((1, RB), -np.inf, f32))

            def weigh(b, c):
                p = jnp.exp2(sc_s[b] - m)
                return (c[0] + jnp.sum(p, axis=0, keepdims=True),
                        c[1] + _dot(pltpu.bitcast(vt_s[b], bf16), p.astype(bf16)))

            l, o = jax.lax.fori_loop(
                0, NB, weigh, (jnp.zeros((1, RB), f32), jnp.zeros((DH, RB), f32)))
            finish(t, l, o)
            return 0

        jax.lax.fori_loop(0, NT, tile, 0)

    for cp in late_copies:
        cp.wait()

    def tail(b, _):
        r0 = pl.multiple_of(b * RB, RB)
        rows = pl.ds(r0, RB)
        g = D // 4
        parts = []
        for j, sh in enumerate((1, -1, 2, -2)):
            win = h_s[pl.ds(r0, RB + 2 * PAD), j * g:(j + 1) * g]
            parts.append(win[PAD - sh:PAD - sh + RB, :].astype(bf16))
        x1 = xn_s[rows, :] + _dot(jnp.concatenate(parts, axis=-1), w2_v[...])
        s = jax.lax.dot_general(ot_s[b], wo_v[...], _TN_DIMS, preferred_element_type=f32)
        hid = _gelu(_dot(_ln(x1).astype(bf16), w3_v[...])).astype(bf16)
        y = x1 + _dot(hid, w4_v[...])
        gate = y * jax.nn.sigmoid(y)
        out_v[rows, :] = (x_v[rows, :].astype(f32) + s * gate).astype(bf16)
        o_copy(b).start()
        return 0

    jax.lax.fori_loop(0, NB, tail, 0)
    for b in range(NB):
        o_copy(b).wait()


@jax.jit
def pallas_recurrent_scan__grouped_kv_mqa__mixer_s_mlp__prompt_kernel(
    A_x: jax.Array,
    A_wq: jax.Array,
    A_wk: jax.Array,
    A_wv: jax.Array,
    A_wo: jax.Array,
    B_x: jax.Array,
    B_w1: jax.Array,
    B_w2: jax.Array,
    B_w3: jax.Array,
    B_w4: jax.Array,
):
    del B_x
    vm = pltpu.VMEM
    out = pl.pallas_call(
        _kernel,
        out_shape=jax.ShapeDtypeStruct((S, D), bf16),
        in_specs=[pl.BlockSpec(memory_space=pl.ANY)] * 9,
        out_specs=pl.BlockSpec(memory_space=pl.ANY),
        scratch_shapes=[
            vm((S, D), bf16), vm((D, D), bf16), vm((DH, D), bf16), vm((DH, D), bf16),
            vm((D, D), bf16), vm((D, D), bf16), vm((D, D), bf16), vm((D, F), bf16),
            vm((F, D), bf16), vm((S, D), bf16),
            vm((D + 2 * DH, D), bf16),
            vm((S, D), f32),
            vm((S + 2 * PAD, D), f32),
            vm((S // 2, 128), u32),
            vm((NB, DH // 2, RB), u32),
            vm((NB, D, RB), bf16),
            vm((NB, D, RB), bf16),
            vm((2, DH, 8, RB), f32),
            vm((DH, NG * 8, 128), f32),
            vm((LAG, CK // 2, RB), u32),
            vm((NB, RB, RB), f32),
            pltpu.SemaphoreType.DMA((NB,)),
            pltpu.SemaphoreType.DMA((8,)),
            pltpu.SemaphoreType.DMA((NB,)),
        ],
        compiler_params=pltpu.CompilerParams(vmem_limit_bytes=100 * 1024 * 1024),
    )(A_x.reshape(S, D), A_wq, A_wk.T, A_wv.T, A_wo, B_w1, B_w2, B_w3, B_w4)
    return out.reshape(A_x.shape)
```
